```python
import os as _os
_os.environ.setdefault("JAX_PLATFORMS", "cpu")
import jax
import jax.numpy as jnp

def _softmax(x, axis=-1):
    return jax.nn.softmax(x, axis=axis)
def _gelu(x):
    return jax.nn.gelu(x, approximate=True)
def _silu(x):
    return jax.nn.silu(x)
def _sigmoid(x):
    return jax.nn.sigmoid(x)
def _layernorm(x, axis=-1, eps=1e-5):
    m = jnp.mean(x, axis=axis, keepdims=True)
    v = jnp.var(x, axis=axis, keepdims=True)
    return (x - m) / jnp.sqrt(v + eps)
def _scatter_add(tgt, idx, src, axis=0):
    return tgt.at[idx].add(src)
def _segment_sum(src, seg, n):
    return jax.ops.segment_sum(src, seg, n)
class _Rng:
    def __init__(self, key):
        self._k = key
    def _next(self):
        self._k, sub = jax.random.split(self._k)
        return sub
    def normal(self, shape):
        return jax.random.normal(self._next(), shape, dtype=jnp.bfloat16)
    def randint(self, lo, hi, shape):
        return jax.random.randint(self._next(), shape, lo, hi, dtype=jnp.int32)
    def uniform(self, shape, lo=0.0, hi=1.0):
        return jax.random.uniform(self._next(), shape, jnp.bfloat16, lo, hi)
    def permutation(self, n):
        return jax.random.permutation(self._next(), n)


kernel_name = 'sequential_preLN__ssm_conv_h3__mixer_channel_mlp__prompt'

def setup_inputs():
    _rng = _Rng(jax.random.key(int.from_bytes(__import__("os").urandom(4), "little")))
    _w = (lambda a: (lambda t: t.astype(jnp.bfloat16) if jnp.issubdtype(t.dtype, jnp.floating) else t)(jnp.asarray(a)))
    def _A_setup():
        B, S, D = 1, 2048, 448
        ks = 4
        return {
            "q": _w((lambda *s: _rng.normal(s) * 0.05)(B, S, D)),
            "k": _w((lambda *s: _rng.normal(s) * 0.05)(B, S, D)),
            "v": _w((lambda *s: _rng.normal(s) * 0.05)(B, S, D)),
            "shift_k": _w((lambda *s: _rng.normal(s) * 0.05)(D, ks) * 0.5),
            "ssm_k": _w((lambda *s: _rng.normal(s) * 0.05)(D, S) * (1.0 / S ** 0.5)),
            "ssm_D": _w((lambda *s: _rng.normal(s) * 0.05)(D)),
        }
    _A_in = _A_setup()

    def _B_setup():
        B, S, D, F = 1, 2048, 448, 1792
        return {
            "x": _w((lambda *s: _rng.normal(s) * 0.05)(B, S, D)),
            "w1": _w((lambda *s: _rng.normal(s) * 0.2)(D, F) * (D ** -0.5)),
            "b1": _w((lambda *s: _rng.normal(s) * 0.2)(F)),
            "w2": _w((lambda *s: _rng.normal(s) * 0.2)(F, D) * (F ** -0.5)),
            "b2": _w((lambda *s: _rng.normal(s) * 0.05)(D)),
        }
    _B_in = _B_setup()

    return {
        "A_q": _A_in["q"],
        "A_k": _A_in["k"],
        "A_v": _A_in["v"],
        "A_shift_k": _A_in["shift_k"],
        "A_ssm_k": _A_in["ssm_k"],
        "A_ssm_D": _A_in["ssm_D"],
        "B_x": _B_in["x"],
        "B_w1": _B_in["w1"],
        "B_b1": _B_in["b1"],
        "B_w2": _B_in["w2"],
        "B_b2": _B_in["b2"],
    }

def reference(A_q, A_k, A_v, A_shift_k, A_ssm_k, A_ssm_D, B_x, B_w1, B_b1, B_w2, B_b2):
    def _A_ref(q, k, v, shift_k, ssm_k, ssm_D):
        B, S, D = q.shape
        ks = shift_k.shape[-1]
        k_pad = jnp.pad(k, ((0, 0), (ks - 1, 0), (0, 0)))
        k_shift = jnp.zeros_like(k)
        for t in range(ks):
            k_shift = k_shift + k_pad[:, t:t + S, :] * shift_k[:, ks - 1 - t][None, None, :]
        kv = k_shift * v
        L = 2 * S
        kv_pad = jnp.pad(kv, ((0, 0), (0, S), (0, 0)))
        kf_pad = jnp.pad(ssm_k, ((0, 0), (0, S)))
        kv_f = (lambda x, axes=(-2,-1): jnp.fft.rfft2(x.astype(jnp.float32), axes=axes))(kv_pad[:, None, :, :], axes=(1, 2))
        kf_f = (lambda x, axes=(-2,-1): jnp.fft.rfft2(x.astype(jnp.float32), axes=axes))(kf_pad[:, None, :], axes=(1, 2))
        kf_f = (lambda x, *d: x.transpose(*d))(kf_f, 1, 2, 0)
        y_f = kv_f * kf_f[None, :, :, :]
        y = (lambda x, s, axes=(-2,-1): jnp.fft.irfft2(x, s=s, axes=axes).astype(jnp.bfloat16))(y_f, (1, L), axes=(1, 2))[:, 0, :S, :]
        y = y + kv * ssm_D[None, None, :]
        return q * y

    def _B_ref(x, w1, b1, w2, b2):
        y = _layernorm(x, axis=-1)
        h = _gelu(jnp.einsum("bsd,df->bsf", y, w1) + b1)
        return jnp.einsum("bsf,fd->bsd", h, w2) + b2

    x = A_q
    h = x + _A_ref(_layernorm(x, axis=-1), A_k, A_v, A_shift_k, A_ssm_k, A_ssm_D)
    h2 = h + _B_ref(_layernorm(h, axis=-1), B_w1, B_b1, B_w2, B_b2)
    return h2
```

```python
import os
import numpy as np
import jax
import jax.numpy as jnp
import jax.experimental.pallas as pl
import jax.experimental.pallas.tpu as pltpu

S, D, F, KS = 2048, 448, 1792, 4
DP = 512
B = 128
NB = S // B
TM = 256
NC = S // TM
BPC = TM // B
f32, bf16 = jnp.float32, jnp.bfloat16

def _dft_mats():
    f = np.arange(B)[None, :] + 0.5
    t = np.arange(B)[:, None]
    ang = 2 * np.pi * f * t / (2 * B)
    fwd = np.concatenate([np.cos(ang), -np.sin(ang)], 1)
    inv = np.concatenate([np.cos(ang).T, -np.sin(ang).T], 0) / B
    return np.concatenate([fwd, inv.T], 0).astype(np.float32)

def _ln0(x):
    m = jnp.sum(x, 0, keepdims=True) * (1.0 / D)
    c = x - m
    v = jnp.sum(c * c, 0, keepdims=True) * (1.0 / D)
    return c * jax.lax.rsqrt(v + 1e-5)

def _gelu(z):
    c = 0.7978845608028654
    u = z * (z * z * (c * 0.044715) + c)
    hz = 0.5 * z
    return hz * jnp.tanh(u) + hz

def _col(ref):
    r = ref[...].astype(f32).reshape(1, -1)
    return jnp.transpose(jnp.broadcast_to(r, (128, r.shape[1])))

def _kernel(q_h, k_h, v_h, sk_h, ssm_h, d_h, w1_h, b1_h, w2_h, b2_h, dft_h, o_h,
            q_v, k_v, v_v, sk_v, ssm_v, d_v, w1_v, b1_v, w2_v, b2_v, dft_v, o_v,
            w1t_v, a_v, b2c_v, X_v, K_v, Z_v, sems, osem):
    cps = {}
    n = [0]
    def start(name, src, dst):
        c = pltpu.make_async_copy(src, dst, sems.at[n[0]]); n[0] += 1
        c.start(); cps[name] = c
    half = lambda r, c: r.at[:, pl.ds(c * TM, TM)]
    start('dft', dft_h, dft_v); start('sk', sk_h, sk_v); start('d', d_h, d_v)
    for c in range(NC):
        start(('s', c), half(ssm_h, c), half(ssm_v, c))
        start(('k', c), half(k_h, c), half(k_v, c)); start(('v', c), half(v_h, c), half(v_v, c))
    start('w1', w1_h, w1_v.at[pl.ds(0, D)]); start('b1', b1_h, b1_v)
    start('q', q_h, q_v); start('w2', w2_h, w2_v); start('b2', b2_h, b2_v)

    cps['dft'].wait(); cps['sk'].wait(); cps['d'].wait()
    fwd = dft_v[0:B, :]
    sk = sk_v[...].astype(f32)
    taps = [jnp.transpose(jnp.broadcast_to(sk[t:t + 1], (128, D))) for t in range(KS)]
    dcol = _col(d_v)
    lane = jax.lax.broadcasted_iota(jnp.int32, (D, B), 1)
    sgn = (1 - 2 * (lane & 1)).astype(f32)
    prev = None; kprev = None
    for j in range(NB):
        if j % BPC == 0:
            for nm in 'skv': cps[(nm, j // BPC)].wait()
        cs = slice(j * B, (j + 1) * B)
        s = jnp.dot(ssm_v[:, cs], fwd, preferred_element_type=f32)
        re, im = s[:, :B], s[:, B:]
        if prev is None:
            c_, d_ = re + dcol, im
        else:
            c_, d_ = re - sgn * prev[1], im + sgn * prev[0]
        prev = (re, im)
        K_v[j, 0] = c_; K_v[j, 1] = d_ - c_; K_v[j, 2] = c_ + d_
        kc = k_v[:, cs].astype(f32)
        ksh = kc * taps[0]
        for t in range(1, KS):
            r = pltpu.roll(kc, t, 1)
            p = 0.0 if kprev is None else kprev[t - 1]
            ksh = ksh + jnp.where(lane >= t, r, p) * taps[t]
        kprev = [pltpu.roll(kc, t, 1) for t in range(1, KS)]
        kv = (ksh * v_v[:, cs].astype(f32)).astype(bf16)
        s = jnp.dot(kv, fwd, preferred_element_type=f32)
        a, b = s[:, :B], s[:, B:]
        X_v[j, 0] = a + b; X_v[j, 1] = a; X_v[j, 2] = b

    def mac(r, _):
        rows = pl.ds(pl.multiple_of(r * 16, 16), 16)
        for i0 in range(0, NB, 2):
            acc = {}
            for j in range(i0 + 2):
                for p in range(3):
                    x = X_v[j, p, rows, :]
                    for i in (i0, i0 + 1):
                        if j > i: continue
                        t = x * K_v[i - j, p, rows, :]
                        acc[i, p] = t if (i, p) not in acc else acc[i, p] + t
            for i in (i0, i0 + 1):
                Z_v[i, rows, 0:B] = (acc[i, 0] - acc[i, 2]).astype(bf16)
                Z_v[i, rows, B:2 * B] = (acc[i, 0] + acc[i, 1]).astype(bf16)
        return 0
    jax.lax.fori_loop(0, D // 16, mac, 0)

    cps['w1'].wait(); cps['b1'].wait()
    row = jax.lax.broadcasted_iota(jnp.int32, (DP - D, F), 0)
    w1_v[D:DP, :] = jnp.where(row == 0, b1_v[...].astype(f32).reshape(1, F), 0.0).astype(bf16)
    for fc in range(F // 128):
        w1t_v[fc * 128:(fc + 1) * 128, :] = jnp.transpose(w1_v[:, fc * 128:(fc + 1) * 128])
    row = jax.lax.broadcasted_iota(jnp.int32, (DP - D, TM), 0)
    a_v[D:DP, :] = jnp.where(row == 0, 1.0, 0.0).astype(bf16)
    cps['q'].wait(); cps['w2'].wait(); cps['b2'].wait()
    b2c_v[...] = _col(b2_v)
    inv = jnp.transpose(dft_v[B:2 * B, :])
    def chunk(c, _):
        c0 = pl.multiple_of(c * TM, TM)
        cs = pl.ds(c0, TM)
        y = jnp.concatenate([jnp.dot(Z_v[c * BPC + jj], inv, preferred_element_type=f32) for jj in range(BPC)], 1)
        x = q_v[:, cs].astype(f32)
        h = x + _ln0(x) * y
        a_v[0:D, :] = _ln0(h).astype(bf16)
        z = jnp.dot(w1t_v[...], a_v[...], preferred_element_type=f32)
        g = _gelu(z).astype(bf16)
        o = jnp.dot(w2_v[...], g, preferred_element_type=f32) + h + jnp.concatenate([b2c_v[...]] * BPC, 1)
        o_v[:, cs] = o.astype(bf16)
        pltpu.make_async_copy(o_v.at[:, cs], o_h.at[:, cs], osem.at[c]).start()
        return 0
    jax.lax.fori_loop(0, NC, chunk, 0)
    for c in range(NC):
        pltpu.make_async_copy(half(o_v, c), half(o_h, c), osem.at[c]).wait()

_DFT = _dft_mats()

@jax.jit
def pallas_sequential_preLN__ssm_conv_h3__mixer_channel_mlp__prompt_kernel(
    A_q, A_k, A_v, A_shift_k, A_ssm_k, A_ssm_D, B_x, B_w1, B_b1, B_w2, B_b2):
    del B_x
    ins = (A_q[0].T, A_k[0].T, A_v[0].T, A_shift_k.T, A_ssm_k, A_ssm_D, B_w1, B_b1, B_w2.T, B_b2,
           jnp.asarray(_DFT, bf16))
    vm = lambda a, dt=bf16: pltpu.VMEM(a, dt)
    shp = [a.shape for a in ins]; shp[6] = (DP, F)
    out = pl.pallas_call(
        _kernel,
        out_shape=pltpu.HBM((D, S), bf16),
        in_specs=[pl.BlockSpec(memory_space=pltpu.HBM)] * len(ins),
        out_specs=pl.BlockSpec(memory_space=pltpu.HBM),
        scratch_shapes=[vm(s) for s in shp] + [vm((D, S)), vm((F, DP)), vm((DP, TM)), vm((D, B), f32),
                        vm((NB, 3, D, B), f32), vm((NB, 3, D, B), f32), vm((NB, D, 2 * B)),
                        pltpu.SemaphoreType.DMA((40,)), pltpu.SemaphoreType.DMA((NC,))],
        compiler_params=pltpu.CompilerParams(vmem_limit_bytes=100 * 1024 * 1024),
    )(*ins)
    return out.T[None]
```

```python
import numpy as np
import jax
import jax.numpy as jnp
import jax.experimental.pallas as pl
import jax.experimental.pallas.tpu as pltpu

S, D, F, KS = 2048, 448, 1792, 4
DP = 512
B = 128
NB = S // B
TM = 256
NC = S // TM
BPC = TM // B
f32, bf16 = jnp.float32, jnp.bfloat16

def _dft_mats():
    f = np.arange(B)[None, :] + 0.5
    t = np.arange(B)[:, None]
    ang = 2 * np.pi * f * t / (2 * B)
    fwd = np.concatenate([np.cos(ang), -np.sin(ang)], 1)
    inv = np.concatenate([np.cos(ang).T, -np.sin(ang).T], 0) / B
    return np.concatenate([fwd, inv.T], 0).astype(np.float32)

def _ln0(x):
    m = jnp.sum(x, 0, keepdims=True) * (1.0 / D)
    c = x - m
    v = jnp.sum(c * c, 0, keepdims=True) * (1.0 / D)
    return c * jax.lax.rsqrt(v + 1e-5)

def _gelu(z):
    c = 0.7978845608028654
    u = z * (z * z * (c * 0.044715) + c)
    hz = 0.5 * z
    return hz * jnp.tanh(u) + hz

def _col(ref):
    r = ref[...].astype(f32).reshape(1, -1)
    return jnp.transpose(jnp.broadcast_to(r, (128, r.shape[1])))

def _kernel(q_h, k_h, v_h, sk_h, ssm_h, d_h, w1_h, b1_h, w2_h, b2_h, dft_h, o_h,
            q_v, k_v, v_v, sk_v, ssm_v, d_v, w1_v, b1_v, w2_v, b2_v, dft_v, o_v,
            w1t_v, a_v, b2c_v, X_v, K_v, Z_v, H_v, sems, osem):
    cps = {}
    n = [0]
    def start(name, src, dst):
        c = pltpu.make_async_copy(src, dst, sems.at[n[0]]); n[0] += 1
        c.start(); cps[name] = c
    half = lambda r, c: r.at[:, pl.ds(c * TM, TM)]
    start('dft', dft_h, dft_v); start('sk', sk_h, sk_v); start('d', d_h, d_v)
    for c in range(NC):
        start(('s', c), half(ssm_h, c), half(ssm_v, c))
        start(('k', c), half(k_h, c), half(k_v, c)); start(('v', c), half(v_h, c), half(v_v, c))
    start('w1', w1_h, w1_v.at[pl.ds(0, D)]); start('b1', b1_h, b1_v)
    start('q', q_h, q_v); start('w2', w2_h, w2_v); start('b2', b2_h, b2_v)

    cps['dft'].wait(); cps['sk'].wait(); cps['d'].wait()
    fwd = dft_v[0:B, :]
    sk = sk_v[...].astype(f32)
    taps = [jnp.transpose(jnp.broadcast_to(sk[t:t + 1], (128, D))) for t in range(KS)]
    dcol = _col(d_v)
    lane = jax.lax.broadcasted_iota(jnp.int32, (D, B), 1)
    sgn = (1 - 2 * (lane & 1)).astype(f32)
    prev = None; kprev = None
    for j in range(NB):
        if j % BPC == 0:
            for nm in 'skv': cps[(nm, j // BPC)].wait()
        cs = slice(j * B, (j + 1) * B)
        s = jnp.dot(ssm_v[:, cs], fwd, preferred_element_type=f32)
        re, im = s[:, :B], s[:, B:]
        if prev is None:
            c_, d_ = re + dcol, im
        else:
            c_, d_ = re - sgn * prev[1], im + sgn * prev[0]
        prev = (re, im)
        K_v[j, 0] = c_; K_v[j, 1] = d_ - c_; K_v[j, 2] = c_ + d_
        kc = k_v[:, cs].astype(f32)
        ksh = kc * taps[0]
        if j: kp = k_v[:, (j - 1) * B:j * B].astype(f32)
        for t in range(1, KS):
            m = jnp.where(lane >= B - t, kp if j else 0.0, kc)
            ksh = ksh + pltpu.roll(m, t, 1) * taps[t]
        kv = (ksh * v_v[:, cs].astype(f32)).astype(bf16)
        s = jnp.dot(kv, fwd, preferred_element_type=f32)
        a, b = s[:, :B], s[:, B:]
        X_v[j, 0] = a + b; X_v[j, 1] = a; X_v[j, 2] = b

    cps['w1'].wait(); cps['b1'].wait()
    row = jax.lax.broadcasted_iota(jnp.int32, (DP - D, F), 0)
    w1_v[D:DP, :] = jnp.where(row == 0, b1_v[...].astype(f32).reshape(1, F), 0.0).astype(bf16)
    for fc in range(F // 128):
        w1t_v[fc * 128:(fc + 1) * 128, :] = jnp.transpose(w1_v[:, fc * 128:(fc + 1) * 128])
    def mac(r, _):
        NO = 4
        for hh in range(2):
          rows = pl.ds(pl.multiple_of(r * 16 + hh * 8, 8), 8)
          for i0 in range(0, NB, NO):
            acc = {}
            for j in range(i0 + NO):
                for p in range(3):
                    x = X_v[j, p, rows, :]
                    for i in range(i0, i0 + NO):
                        if j > i: continue
                        t = x * K_v[i - j, p, rows, :]
                        acc[i, p] = t if (i, p) not in acc else acc[i, p] + t
            for i in range(i0, i0 + NO):
                Z_v[i, rows, 0:B] = acc[i, 0] - acc[i, 2]
                Z_v[i, rows, B:2 * B] = acc[i, 0] + acc[i, 1]
        return 0
    jax.lax.fori_loop(0, D // 16, mac, 0)

    row = jax.lax.broadcasted_iota(jnp.int32, (DP - D, TM), 0)
    for u in range(2): a_v[u, D:DP, :] = jnp.where(row == 0, 1.0, 0.0).astype(bf16)
    cps['q'].wait(); cps['w2'].wait(); cps['b2'].wait()
    b2c_v[...] = _col(b2_v)
    inv = jnp.transpose(dft_v[B:2 * B, :])
    def prep(c, slot):
        cs = pl.ds(pl.multiple_of(c * TM, TM), TM)
        y = jnp.concatenate([jnp.dot(Z_v[c * BPC + jj].astype(bf16), inv, preferred_element_type=f32) for jj in range(BPC)], 1)
        x = q_v[:, cs].astype(f32)
        h = x + _ln0(x) * y
        H_v[slot] = h + jnp.concatenate([b2c_v[...]] * BPC, 1)
        a_v[slot, 0:D, :] = _ln0(h).astype(bf16)
    def mlp(c, slot):
        cs = pl.ds(pl.multiple_of(c * TM, TM), TM)
        z = jnp.dot(w1t_v[...], a_v[slot], preferred_element_type=f32)
        g = _gelu(z).astype(bf16)
        o = jnp.dot(w2_v[...], g, preferred_element_type=f32) + H_v[slot]
        o_v[:, cs] = o.astype(bf16)
        pltpu.make_async_copy(o_v.at[:, cs], o_h.at[:, cs], osem.at[c]).start()
    prep(0, 0)
    def chunk(cc, _):
        c = 2 * cc
        prep(c + 1, 1)
        mlp(c, 0)
        prep(jnp.minimum(c + 2, NC - 1), 0)
        mlp(c + 1, 1)
        return 0
    jax.lax.fori_loop(0, NC // 2, chunk, 0)
    for c in range(NC):
        pltpu.make_async_copy(half(o_v, c), half(o_h, c), osem.at[c]).wait()

_DFT = _dft_mats()

@jax.jit
def pallas_sequential_preLN__ssm_conv_h3__mixer_channel_mlp__prompt_kernel(
    A_q, A_k, A_v, A_shift_k, A_ssm_k, A_ssm_D, B_x, B_w1, B_b1, B_w2, B_b2):
    del B_x
    ins = (A_q[0].T, A_k[0].T, A_v[0].T, A_shift_k.T, A_ssm_k, A_ssm_D, B_w1, B_b1, B_w2.T, B_b2,
           jnp.asarray(_DFT, bf16))
    vm = lambda a, dt=bf16: pltpu.VMEM(a, dt)
    shp = [a.shape for a in ins]; shp[6] = (DP, F)
    out = pl.pallas_call(
        _kernel,
        out_shape=pltpu.HBM((D, S), bf16),
        in_specs=[pl.BlockSpec(memory_space=pltpu.HBM)] * len(ins),
        out_specs=pl.BlockSpec(memory_space=pltpu.HBM),
        scratch_shapes=[vm(s) for s in shp] + [vm((D, S)), vm((F, DP)), vm((2, DP, TM)), vm((D, B), f32),
                        vm((NB, 3, D, B), f32), vm((NB, 3, D, B), f32), vm((NB, D, 2 * B), f32), vm((2, D, TM), f32),
                        pltpu.SemaphoreType.DMA((40,)), pltpu.SemaphoreType.DMA((NC,))],
        compiler_params=pltpu.CompilerParams(vmem_limit_bytes=100 * 1024 * 1024),
    )(*ins)
    return out.T[None]
```
